```python
import jax
import jax.numpy as jnp

def _softmax(x, axis=-1):
    return jax.nn.softmax(x, axis=axis)
def _gelu(x):
    return jax.nn.gelu(x, approximate=True)
def _silu(x):
    return jax.nn.silu(x)
def _sigmoid(x):
    return jax.nn.sigmoid(x)
def _layernorm(x, axis=-1, eps=1e-5):
    m = jnp.mean(x, axis=axis, keepdims=True)
    v = jnp.var(x, axis=axis, keepdims=True)
    return (x - m) / jnp.sqrt(v + eps)
def _scatter_add(tgt, idx, src, axis=0):
    return tgt.at[idx].add(src)
def _segment_sum(src, seg, n):
    return jax.ops.segment_sum(src, seg, n)
class _Rng:
    def __init__(self, key):
        self._k = key
    def _next(self):
        self._k, sub = jax.random.split(self._k)
        return sub
    def normal(self, shape):
        return jax.random.normal(self._next(), shape, dtype=jnp.bfloat16)
    def randint(self, lo, hi, shape):
        return jax.random.randint(self._next(), shape, lo, hi, dtype=jnp.int32)
    def uniform(self, shape, lo=0.0, hi=1.0):
        return jax.random.uniform(self._next(), shape, jnp.bfloat16, lo, hi)
    def permutation(self, n):
        return jax.random.permutation(self._next(), n)


kernel_name = 'gated_mix__sliding_local_dilated__glu_gated_reglu__prompt'

def setup_inputs():
    _rng = _Rng(jax.random.key(int.from_bytes(__import__("os").urandom(4), "little")))
    _w = (lambda a: (lambda t: t.astype(jnp.bfloat16) if jnp.issubdtype(t.dtype, jnp.floating) else t)(jnp.asarray(a)))
    def _A_setup():
        B, S, D = 1, 2048, 1024
        return {
            "x": _w((lambda *s: _rng.normal(s) * 0.05)(B, S, D)),
            "wqkv": _w((lambda *s: _rng.normal(s) * 0.05)(D, 3 * D)),
            "wo": _w((lambda *s: _rng.normal(s) * 0.05)(D, D)),
        }
    _A_in = _A_setup()

    def _B_setup():
        B, S, D, F = 1, 2048, 1024, 3584
        return {
            "x": _w((lambda *s: _rng.normal(s) * 0.05)(B, S, D)),
            "W_gate": _w((lambda *s: _rng.normal(s) * 0.05)(D, F) * (2.0 / D) ** 0.5),
            "W_up": _w((lambda *s: _rng.normal(s) * 0.05)(D, F) * (2.0 / D) ** 0.5),
            "W_down": _w((lambda *s: _rng.normal(s) * 0.05)(F, D) * (1.0 / F) ** 0.5),
        }
    _B_in = _B_setup()

    return {
        "A_x": _A_in["x"],
        "A_wqkv": _A_in["wqkv"],
        "A_wo": _A_in["wo"],
        "B_x": _B_in["x"],
        "B_W_gate": _B_in["W_gate"],
        "B_W_up": _B_in["W_up"],
        "B_W_down": _B_in["W_down"],
        "gate_w": _w((lambda *s: _rng.normal(s) * 0.05)(1024)),
    }

def reference(A_x, A_wqkv, A_wo, B_x, B_W_gate, B_W_up, B_W_down, gate_w):
    def _A_ref(x, wqkv, wo):
        B, S, D = x.shape
        H = 32; Dh = D // H
        W, dil = 8, 2
        qkv = (lambda x, *d: x.transpose(*d))((x @ wqkv).reshape(B, S, 3, H, Dh), 2, 0, 3, 1, 4)
        q, k, v = qkv[0], qkv[1], qkv[2]
        scale = Dh ** -0.5
        pos = jnp.arange(S)
        off = jnp.arange(W) * dil
        idx = pos[:, None] - off[None, :]
        mask = idx >= 0
        idx_c = jnp.where(mask, idx, 0).reshape(-1)
        kg = k[:, :, idx_c, :].reshape(B, H, S, W, Dh)
        vg = v[:, :, idx_c, :].reshape(B, H, S, W, Dh)
        logits = jnp.einsum("bhsd,bhswd->bhsw", q, kg) * scale
        logits = jnp.where(mask[None, None, :, :], logits, -1e9)
        attn = _softmax(logits, axis=-1)
        o = jnp.einsum("bhsw,bhswd->bhsd", attn, vg)
        return (lambda x, *d: x.transpose(*d))(o, 0, 2, 1, 3).reshape(B, S, D) @ wo

    def _B_ref(x, W_gate, W_up, W_down):
        gate = jnp.einsum("bsd,df->bsf", x, W_gate)
        up = jnp.einsum("bsd,df->bsf", x, W_up)
        gate = gate * (lambda x, dt: x.astype(dt))(gate > 0, gate.dtype)
        h = gate * up
        return jnp.einsum("bsf,fd->bsd", h, W_down)

    x = A_x
    g = _sigmoid((x * gate_w).sum(-1, keepdims=True))
    a = _A_ref(x, A_wqkv, A_wo)
    b = _B_ref(x, B_W_gate, B_W_up, B_W_down)
    return g * a + (1 - g) * b
```

```python
import functools
import jax
import jax.numpy as jnp
import numpy as np
import jax.experimental.pallas as pl
import jax.experimental.pallas.tpu as pltpu

_H, _W, _DIL = 32, 8, 2
_F32, _BF16 = jnp.float32, jnp.bfloat16


def _dot(a, b):
    return jnp.dot(a, b, preferred_element_type=_F32)


def _kernel(x_ref, gw_ref, wqkv_hbm, wo_hbm, wg_hbm, wu_hbm, wd_hbm, out_ref,
            wqkv, wo, wg, wu, wd, kt_ref, vt_ref, ot_ref, h_ref, sems, *, T, D, F, NG, fch):
    i = pl.program_id(0)
    G = D // NG
    Dh = D // _H
    scale = Dh ** -0.5
    foff = np.concatenate([[0], np.cumsum(fch)]).tolist()

    def cp_qkv(g, j):
        c = pl.ds(j * D + g * G, G)
        return pltpu.make_async_copy(wqkv_hbm.at[:, c], wqkv.at[:, c], sems.at[g * 5 + j])

    def cp_g(g):
        c = pl.ds(foff[g], fch[g])
        return pltpu.make_async_copy(wg_hbm.at[:, c], wg.at[:, c], sems.at[g * 5 + 3])

    def cp_u(g):
        c = pl.ds(foff[g], fch[g])
        return pltpu.make_async_copy(wu_hbm.at[:, c], wu.at[:, c], sems.at[g * 5 + 4])

    cp_o = pltpu.make_async_copy(wo_hbm, wo, sems.at[NG * 5])
    cp_d = pltpu.make_async_copy(wd_hbm, wd, sems.at[NG * 5 + 1])

    @pl.when(i == 0)
    def _():
        for g in range(NG):
            for j in (1, 2, 0):
                cp_qkv(g, j).start()
            cp_g(g).start()
            cp_u(g).start()
        cp_d.start()
        cp_o.start()
        kt_ref[:, 0:128] = jnp.zeros((D, 128), kt_ref.dtype)
        vt_ref[:, 0:128] = jnp.zeros((D, 128), vt_ref.dtype)

    x = x_ref[...]
    pos = i * T + jax.lax.broadcasted_iota(jnp.int32, (1, 1, T), 2)

    for g in range(NG):
        @pl.when(i == 0)
        def _():
            for j in range(3):
                cp_qkv(g, j).wait()
            cp_g(g).wait()
            cp_u(g).wait()

        rows = slice(g * G, (g + 1) * G)
        k = _dot(x, wqkv[:, D + g * G: D + (g + 1) * G])
        kt_ref[rows, 128:128 + T] = k.T
        v = _dot(x, wqkv[:, 2 * D + g * G: 2 * D + (g + 1) * G])
        vt_ref[rows, 128:128 + T] = v.T
        qt = (_dot(x, wqkv[:, g * G:(g + 1) * G]) * scale).T

        fc = slice(foff[g], foff[g + 1])
        ga = _dot(x, wg[:, fc])
        up = _dot(x, wu[:, fc])
        h_ref[:, fc] = (ga * (ga > 0).astype(_F32) * up).astype(_BF16)

        nh = G // Dh
        logits = []
        for w in range(_W):
            ks = kt_ref[rows, 128 - _DIL * w: 128 - _DIL * w + T]
            l = jnp.sum((qt * ks).reshape(nh, Dh, T), axis=1, keepdims=True)
            if w > 0:
                l = jnp.where(pos >= _DIL * w, l, -1e9)
            logits.append(l)
        m = functools.reduce(jnp.maximum, logits)
        es = [jnp.exp(l - m) for l in logits]
        inv = 1.0 / functools.reduce(lambda a, b: a + b, es)
        acc = None
        for w in range(_W):
            vs = vt_ref[rows, 128 - _DIL * w: 128 - _DIL * w + T].reshape(nh, Dh, T)
            t = es[w] * vs
            acc = t if acc is None else acc + t
        o = (acc * inv).reshape(G, T)
        ot_ref[:, rows] = o.T.astype(_BF16)
        kt_ref[rows, 0:128] = kt_ref[rows, T:T + 128]
        vt_ref[rows, 0:128] = vt_ref[rows, T:T + 128]

    @pl.when(i == 0)
    def _():
        cp_d.wait()
        cp_o.wait()

    gate = jax.nn.sigmoid(jnp.sum(x.astype(_F32) * gw_ref[...].astype(_F32), axis=-1, keepdims=True))
    NC = 512
    for n in range(D // NC):
        c = slice(n * NC, (n + 1) * NC)
        b = _dot(h_ref[...], wd[:, c])
        a = _dot(ot_ref[...], wo[:, c])
        out_ref[:, c] = (gate * a + (1.0 - gate) * b).astype(out_ref.dtype)


@functools.partial(jax.jit, static_argnames=("T", "NG"))
def pallas_gated_mix__sliding_local_dilated__glu_gated_reglu__prompt_kernel(
    A_x, A_wqkv, A_wo, B_x, B_W_gate, B_W_up, B_W_down, gate_w, T=512, NG=8,
):
    del B_x
    B, S, D = A_x.shape
    F = B_W_gate.shape[1]
    nt = F // 128
    fch = tuple(128 * (nt // NG + (1 if g < nt % NG else 0)) for g in range(NG))
    x = A_x.reshape(S, D)
    gw = gate_w.reshape(1, D)
    hbm = pl.BlockSpec(memory_space=pl.ANY)
    out = pl.pallas_call(
        functools.partial(_kernel, T=T, D=D, F=F, NG=NG, fch=fch),
        grid=(S // T,),
        in_specs=[pl.BlockSpec((T, D), lambda i: (i, 0)),
                  pl.BlockSpec((1, D), lambda i: (0, 0)),
                  hbm, hbm, hbm, hbm, hbm],
        out_specs=pl.BlockSpec((T, D), lambda i: (i, 0)),
        out_shape=jax.ShapeDtypeStruct((S, D), A_x.dtype),
        scratch_shapes=[
            pltpu.VMEM((D, 3 * D), _BF16), pltpu.VMEM((D, D), _BF16),
            pltpu.VMEM((D, F), _BF16), pltpu.VMEM((D, F), _BF16), pltpu.VMEM((F, D), _BF16),
            pltpu.VMEM((D, 128 + T), _F32), pltpu.VMEM((D, 128 + T), _F32),
            pltpu.VMEM((T, D), _BF16), pltpu.VMEM((T, F), _BF16),
            pltpu.SemaphoreType.DMA((NG * 5 + 2,)),
        ],
        compiler_params=pltpu.CompilerParams(
            dimension_semantics=("arbitrary",), vmem_limit_bytes=100 * 1024 * 1024),
    )(x, gw, A_wqkv, A_wo, B_W_gate, B_W_up, B_W_down)
    return out.reshape(B, S, D)
```

```python
import functools
import jax
import jax.numpy as jnp
import jax.experimental.pallas as pl
import jax.experimental.pallas.tpu as pltpu

_H, _W, _DIL = 32, 8, 2
_HALO = 128
_F32, _BF16 = jnp.float32, jnp.bfloat16


def _dot(a, b):
    return jnp.dot(a, b, preferred_element_type=_F32)


def _kernel(gw_ref, x_hbm, wqkv_hbm, wo_hbm, wg_hbm, wu_hbm, wd_hbm, out_hbm,
            x, wqkv, wo, wg, wu, wd, kt, vt, o_buf, h_buf, out_buf,
            x_sem, w_sem, p2_sem, out_sem, *, S, D, F, NG, T1, T2):
    G = D // NG
    FG = F // NG
    Dh = D // _H
    scale = Dh ** -0.5
    nt1, nt2 = S // T1, S // T2

    def cp_x(t):
        r = pl.ds(t * T1, T1)
        return pltpu.make_async_copy(x_hbm.at[r, :], x.at[r, :], x_sem.at[t])

    def cp_qkv(g, j, col=None):
        col = j * D + g * G if col is None else col
        return pltpu.make_async_copy(wqkv_hbm.at[:, pl.ds(col, G)], wqkv.at[g, j], w_sem.at[g * 5 + j])

    def cp_ffn(g, j, col=None):
        col = g * FG if col is None else col
        src, dst = ((wg_hbm, wg), (wu_hbm, wu))[j]
        return pltpu.make_async_copy(src.at[:, pl.ds(col, FG)], dst.at[g], w_sem.at[g * 5 + 3 + j])

    cp_d = pltpu.make_async_copy(wd_hbm, wd, p2_sem.at[0])
    cp_o = pltpu.make_async_copy(wo_hbm, wo, p2_sem.at[1])

    def cp_out(t):
        r = pl.ds(pl.multiple_of(t * T2, T2), T2)
        return pltpu.make_async_copy(out_buf.at[r, :], out_hbm.at[r, :], out_sem.at[t])

    cp_x(0).start()
    for j in (1, 2, 0):
        cp_qkv(0, j).start()
    cp_ffn(0, 0).start()
    cp_ffn(0, 1).start()

    def phase1(it, carry):
        g, t = it // nt1, it % nt1

        @pl.when(g == 0)
        def _():
            cp_x(t).wait()

        @pl.when(t == 0)
        def _():
            for j in range(3):
                cp_qkv(g, j, 0).wait()
            kt[:, 0:_HALO] = jnp.zeros((G, _HALO), _F32)
            vt[:, 0:_HALO] = jnp.zeros((G, _HALO), _F32)

        r = pl.ds(pl.multiple_of(t * T1, T1), T1)
        xt = x[r, :]
        kt[:, _HALO:_HALO + T1] = _dot(xt, wqkv[g, 1]).T
        vt[:, _HALO:_HALO + T1] = _dot(xt, wqkv[g, 2]).T
        qt_all = (_dot(xt, wqkv[g, 0]) * scale).T

        @pl.when(t == 0)
        def _():
            cp_ffn(g, 0, 0).wait()
            cp_ffn(g, 1, 0).wait()
            for gn in range(1, NG):
                @pl.when(g == gn - 1)
                def _():
                    if gn == 1:
                        for tn in range(1, nt1):
                            cp_x(tn).start()
                    for j in (1, 2, 0):
                        cp_qkv(gn, j).start()
                    cp_ffn(gn, 0).start()
                    cp_ffn(gn, 1).start()

            @pl.when(g == NG - 1)
            def _():
                cp_d.start()
                cp_o.start()

        pos = t * T1 + jax.lax.broadcasted_iota(jnp.int32, (1, T1), 1)
        nh = G // Dh
        nsub = 2
        fcols = [128 * c for c in ((FG // 128 + 1) // 2, FG // 128 // 2)]
        f0 = 0
        for s in range(nsub):
            fc = slice(f0, f0 + fcols[s])
            f0 += fcols[s]
            ga = _dot(x[r, :], wg[g, :, fc])
            up = _dot(x[r, :], wu[g, :, fc])
            h_buf[g, r, fc] = (ga * (ga > 0).astype(_F32) * up).astype(_BF16)
            outs = []
            for hh in range(s * nh // nsub, (s + 1) * nh // nsub):
                rows = slice(hh * Dh, (hh + 1) * Dh)
                qt = qt_all[rows]
                logits = []
                for w in range(_W):
                    lo = _HALO - _DIL * w
                    l = jnp.sum(qt * kt[rows, lo:lo + T1], axis=0, keepdims=True)
                    if w > 0:
                        l = jnp.where(pos >= _DIL * w, l, -1e9)
                    logits.append(l)
                m = functools.reduce(jnp.maximum, logits)
                es = [jnp.exp(l - m) for l in logits]
                inv = 1.0 / functools.reduce(lambda a, b: a + b, es)
                acc = None
                for w in range(_W):
                    lo = _HALO - _DIL * w
                    term = es[w] * vt[rows, lo:lo + T1]
                    acc = term if acc is None else acc + term
                outs.append(acc * inv)
                kt[rows, 0:_HALO] = kt[rows, T1:T1 + _HALO]
                vt[rows, 0:_HALO] = vt[rows, T1:T1 + _HALO]
            c0 = s * G // nsub
            o_buf[g, r, c0:c0 + G // nsub] = jnp.concatenate(outs, axis=0).T.astype(_BF16)
        return carry

    jax.lax.fori_loop(0, NG * nt1, phase1, 0)
    cp_d.wait()
    cp_o.wait()

    def phase2(t, carry):
        r = pl.ds(pl.multiple_of(t * T2, T2), T2)
        gate = jax.nn.sigmoid(jnp.sum(
            x[r, :].astype(_F32) * gw_ref[...].astype(_F32)[None, :], axis=-1, keepdims=True))
        NC = 512
        for n in range(D // NC):
            c = slice(n * NC, (n + 1) * NC)
            b = _dot(h_buf[0, r, :], wd[0:FG, c])
            for g in range(1, NG):
                b += _dot(h_buf[g, r, :], wd[g * FG:(g + 1) * FG, c])
            a = _dot(o_buf[0, r, :], wo[0:G, c])
            for g in range(1, NG):
                a += _dot(o_buf[g, r, :], wo[g * G:(g + 1) * G, c])
            out_buf[r, c] = (gate * a + (1.0 - gate) * b).astype(out_buf.dtype)
        cp_out(t).start()
        return carry

    jax.lax.fori_loop(0, nt2, phase2, 0)
    for t in range(nt2):
        cp_out(t).wait()


@functools.partial(jax.jit, static_argnames=("T1", "T2", "NG"))
def pallas_gated_mix__sliding_local_dilated__glu_gated_reglu__prompt_kernel(
    A_x, A_wqkv, A_wo, B_x, B_W_gate, B_W_up, B_W_down, gate_w, T1=512, T2=256, NG=4,
):
    del B_x
    B, S, D = A_x.shape
    F = B_W_gate.shape[1]
    G, FG = D // NG, F // NG
    hbm = pl.BlockSpec(memory_space=pl.ANY)
    vmem = pltpu.VMEM
    out = pl.pallas_call(
        functools.partial(_kernel, S=S, D=D, F=F, NG=NG, T1=T1, T2=T2),
        in_specs=[pl.BlockSpec(memory_space=pltpu.VMEM), hbm, hbm, hbm, hbm, hbm, hbm],
        out_specs=hbm,
        out_shape=jax.ShapeDtypeStruct((S, D), A_x.dtype),
        scratch_shapes=[
            vmem((S, D), _BF16), vmem((NG, 3, D, G), _BF16), vmem((D, D), _BF16),
            vmem((NG, D, FG), _BF16), vmem((NG, D, FG), _BF16), vmem((F, D), _BF16),
            vmem((G, _HALO + T1), _F32), vmem((G, _HALO + T1), _F32),
            vmem((NG, S, G), _BF16), vmem((NG, S, FG), _BF16), vmem((S, D), A_x.dtype),
            pltpu.SemaphoreType.DMA((S // T1,)), pltpu.SemaphoreType.DMA((NG * 5,)),
            pltpu.SemaphoreType.DMA((2,)), pltpu.SemaphoreType.DMA((S // T2,)),
        ],
        compiler_params=pltpu.CompilerParams(vmem_limit_bytes=110 * 1024 * 1024),
    )(gate_w, A_x.reshape(S, D), A_wqkv, A_wo, B_W_gate, B_W_up, B_W_down)
    return out.reshape(B, S, D)
```

```python
import functools
import jax
import jax.numpy as jnp
import jax.experimental.pallas as pl
import jax.experimental.pallas.tpu as pltpu

_H, _W, _DIL = 32, 8, 2
_HALO = 128
_F32, _BF16 = jnp.float32, jnp.bfloat16


def _dot(a, b):
    return jnp.dot(a, b, preferred_element_type=_F32)


def _kernel(gw_ref, x_hbm, wqkv_hbm, wo_hbm, wg_hbm, wu_hbm, wd_hbm, out_hbm,
            x, wqkv, wo, wg, wu, wd, kt, vt, o_buf, h_buf, out_buf,
            x_sem, w_sem, p2_sem, out_sem, *, S, D, F, NG, T1, T2):
    G = D // NG
    FG = F // NG
    Dh = D // _H
    scale = Dh ** -0.5
    nt1, nt2 = S // T1, S // T2

    def cp_x(t):
        r = pl.ds(t * T1, T1)
        return pltpu.make_async_copy(x_hbm.at[r, :], x.at[r, :], x_sem.at[t])

    def cp_qkv(g, j):
        col = j * D + g * G
        return pltpu.make_async_copy(wqkv_hbm.at[:, pl.ds(col, G)], wqkv.at[g, j], w_sem.at[g * 5 + j])

    def cp_ffn(g, j):
        col = g * FG
        src, dst = ((wg_hbm, wg), (wu_hbm, wu))[j]
        return pltpu.make_async_copy(src.at[:, pl.ds(col, FG)], dst.at[g], w_sem.at[g * 5 + 3 + j])

    cp_d = pltpu.make_async_copy(wd_hbm, wd, p2_sem.at[0])
    cp_o = pltpu.make_async_copy(wo_hbm, wo, p2_sem.at[1])

    def cp_out(t):
        r = pl.ds(pl.multiple_of(t * T2, T2), T2)
        return pltpu.make_async_copy(out_buf.at[r, :], out_hbm.at[r, :], out_sem.at[t])

    cp_x(0).start()
    for j in (1, 2, 0):
        cp_qkv(0, j).start()
    cp_ffn(0, 0).start()
    cp_ffn(0, 1).start()

    def phase1(it, carry):
        g, t = it // nt1, it % nt1

        @pl.when(g == 0)
        def _():
            cp_x(t).wait()

        @pl.when(t == 0)
        def _():
            for gs in range(NG):
                @pl.when(g == gs)
                def _():
                    for j in range(3):
                        cp_qkv(gs, j).wait()
            kt[:, 0:_HALO] = jnp.zeros((G, _HALO), _F32)
            vt[:, 0:_HALO] = jnp.zeros((G, _HALO), _F32)

        r = pl.ds(pl.multiple_of(t * T1, T1), T1)
        xt = x[r, :]
        kt[:, _HALO:_HALO + T1] = _dot(xt, wqkv[g, 1]).T
        vt[:, _HALO:_HALO + T1] = _dot(xt, wqkv[g, 2]).T
        qt_all = (_dot(xt, wqkv[g, 0]) * scale).T

        @pl.when(t == 0)
        def _():
            for gn in range(1, NG + 1):
                @pl.when(g == gn - 1)
                def _():
                    cp_ffn(gn - 1, 0).wait()
                    cp_ffn(gn - 1, 1).wait()
                    if gn == NG:
                        cp_d.start()
                        cp_o.start()
                        return
                    if gn == 1:
                        for tn in range(1, nt1):
                            cp_x(tn).start()
                    for j in (1, 2, 0):
                        cp_qkv(gn, j).start()
                    cp_ffn(gn, 0).start()
                    cp_ffn(gn, 1).start()

        pos = t * T1 + jax.lax.broadcasted_iota(jnp.int32, (1, T1), 1)
        nh = G // Dh
        nsub = 2
        fcols = [128 * c for c in ((FG // 128 + 1) // 2, FG // 128 // 2)]
        f0 = 0
        for s in range(nsub):
            fc = slice(f0, f0 + fcols[s])
            f0 += fcols[s]
            ga = _dot(x[r, :], wg[g, :, fc])
            up = _dot(x[r, :], wu[g, :, fc])
            h_buf[g, r, fc] = (ga * (ga > 0).astype(_F32) * up).astype(_BF16)
            outs = []
            for hh in range(s * nh // nsub, (s + 1) * nh // nsub):
                rows = slice(hh * Dh, (hh + 1) * Dh)
                qt = qt_all[rows]
                logits = []
                for w in range(_W):
                    lo = _HALO - _DIL * w
                    l = jnp.sum(qt * kt[rows, lo:lo + T1], axis=0, keepdims=True)
                    if w > 0:
                        l = jnp.where(pos >= _DIL * w, l, -1e9)
                    logits.append(l)
                m = functools.reduce(jnp.maximum, logits)
                es = [jnp.exp(l - m) for l in logits]
                inv = 1.0 / functools.reduce(lambda a, b: a + b, es)
                acc = None
                for w in range(_W):
                    lo = _HALO - _DIL * w
                    term = es[w] * vt[rows, lo:lo + T1]
                    acc = term if acc is None else acc + term
                outs.append(acc * inv)
                kt[rows, 0:_HALO] = kt[rows, T1:T1 + _HALO]
                vt[rows, 0:_HALO] = vt[rows, T1:T1 + _HALO]
            c0 = s * G // nsub
            o_buf[g, r, c0:c0 + G // nsub] = jnp.concatenate(outs, axis=0).T.astype(_BF16)
        return carry

    jax.lax.fori_loop(0, NG * nt1, phase1, 0)
    cp_d.wait()
    cp_o.wait()

    def phase2(t, carry):
        r = pl.ds(pl.multiple_of(t * T2, T2), T2)
        gate = jax.nn.sigmoid(jnp.sum(
            x[r, :].astype(_F32) * gw_ref[...].astype(_F32)[None, :], axis=-1, keepdims=True))
        NC = 512
        for n in range(D // NC):
            c = slice(n * NC, (n + 1) * NC)
            b = _dot(h_buf[0, r, :], wd[0:FG, c])
            for g in range(1, NG):
                b += _dot(h_buf[g, r, :], wd[g * FG:(g + 1) * FG, c])
            a = _dot(o_buf[0, r, :], wo[0:G, c])
            for g in range(1, NG):
                a += _dot(o_buf[g, r, :], wo[g * G:(g + 1) * G, c])
            out_buf[r, c] = (gate * a + (1.0 - gate) * b).astype(out_buf.dtype)
        cp_out(t).start()
        return carry

    jax.lax.fori_loop(0, nt2, phase2, 0)
    for t in range(nt2):
        cp_out(t).wait()


@functools.partial(jax.jit, static_argnames=("T1", "T2", "NG"))
def pallas_gated_mix__sliding_local_dilated__glu_gated_reglu__prompt_kernel(
    A_x, A_wqkv, A_wo, B_x, B_W_gate, B_W_up, B_W_down, gate_w, T1=512, T2=256, NG=4,
):
    del B_x
    B, S, D = A_x.shape
    F = B_W_gate.shape[1]
    G, FG = D // NG, F // NG
    hbm = pl.BlockSpec(memory_space=pl.ANY)
    vmem = pltpu.VMEM
    out = pl.pallas_call(
        functools.partial(_kernel, S=S, D=D, F=F, NG=NG, T1=T1, T2=T2),
        in_specs=[pl.BlockSpec(memory_space=pltpu.VMEM), hbm, hbm, hbm, hbm, hbm, hbm],
        out_specs=hbm,
        out_shape=jax.ShapeDtypeStruct((S, D), A_x.dtype),
        scratch_shapes=[
            vmem((S, D), _BF16), vmem((NG, 3, D, G), _BF16), vmem((D, D), _BF16),
            vmem((NG, D, FG), _BF16), vmem((NG, D, FG), _BF16), vmem((F, D), _BF16),
            vmem((G, _HALO + T1), _F32), vmem((G, _HALO + T1), _F32),
            vmem((NG, S, G), _BF16), vmem((NG, S, FG), _BF16), vmem((S, D), A_x.dtype),
            pltpu.SemaphoreType.DMA((S // T1,)), pltpu.SemaphoreType.DMA((NG * 5,)),
            pltpu.SemaphoreType.DMA((2,)), pltpu.SemaphoreType.DMA((S // T2,)),
        ],
        compiler_params=pltpu.CompilerParams(vmem_limit_bytes=110 * 1024 * 1024),
    )(gate_w, A_x.reshape(S, D), A_wqkv, A_wo, B_W_gate, B_W_up, B_W_down)
    return out.reshape(B, S, D)
```
